```python
import os as _os
_os.environ.setdefault('JAX_PLATFORMS', 'cpu')
import jax
import jax.numpy as jnp

def _softmax(x, axis=-1):
    return jax.nn.softmax(x, axis=axis)

def _gelu(x):
    return jax.nn.gelu(x, approximate=True)

def _silu(x):
    return jax.nn.silu(x)

def _sigmoid(x):
    return jax.nn.sigmoid(x)

def _layernorm(x, axis=-1, eps=1e-05):
    m = jnp.mean(x, axis=axis, keepdims=True)
    v = jnp.var(x, axis=axis, keepdims=True)
    return (x - m) / jnp.sqrt(v + eps)

def _scatter_add(tgt, idx, src, axis=0):
    return tgt.at[idx].add(src)

def _segment_sum(src, seg, n):
    return jax.ops.segment_sum(src, seg, n)

class _Rng:

    def __init__(self, key):
        self._k = key

    def _next(self):
        self._k, sub = jax.random.split(self._k)
        return sub

    def normal(self, shape):
        return jax.random.normal(self._next(), shape, dtype=jnp.bfloat16)

    def randint(self, lo, hi, shape):
        return jax.random.randint(self._next(), shape, lo, hi, dtype=jnp.int32)

    def uniform(self, shape, lo=0.0, hi=1.0):
        return jax.random.uniform(self._next(), shape, jnp.bfloat16, lo, hi)

    def permutation(self, n):
        return jax.random.permutation(self._next(), n)
kernel_name = 'interleave_layers__ssm_conv_h3__mixer_gmlp__prompt'

def setup_inputs():
    _rng = _Rng(jax.random.key(int.from_bytes(__import__("os").urandom(4), "little")))
    _w = lambda a: (lambda t: t.astype(jnp.bfloat16) if jnp.issubdtype(t.dtype, jnp.floating) else t)(jnp.asarray(a))

    def _A_setup():
        B, S, D = (1, 2048, 1024)
        ks = 4
        return {'q': _w((lambda *s: _rng.normal(s) * 0.05)(B, S, D)), 'k': _w((lambda *s: _rng.normal(s) * 1.6)(B, S, D)), 'v': _w((lambda *s: _rng.normal(s) * 1.6)(B, S, D)), 'shift_k': _w((lambda *s: _rng.normal(s) * 1.6)(D, ks) * 0.5), 'ssm_k': _w((lambda *s: _rng.normal(s) * 1.6)(D, S) * (1.0 / S ** 0.5)), 'ssm_D': _w((lambda *s: _rng.normal(s) * 1.6)(D))}
    _A_in = _A_setup()

    def _B_setup():
        B, S, D, F = (1, 2048, 1024, 3584)
        Fh = F // 2
        return {'x': _w((lambda *s: _rng.normal(s) * 0.05)(B, S, D)), 'w_in': _w((lambda *s: _rng.normal(s) * 0.8)(D, 2 * Fh)), 'w_sp': _w(0.01 * (lambda *s: _rng.normal(s) * 0.8)(S, S)), 'b_sp': _w(1.0 + 0.01 * (lambda *s: _rng.normal(s) * 0.2)(S)), 'w_out': _w((lambda *s: _rng.normal(s) * 0.2)(Fh, D))}
    _B_in = _B_setup()
    return {'A_q': _A_in['q'], 'A_k': _A_in['k'], 'A_v': _A_in['v'], 'A_shift_k': _A_in['shift_k'], 'A_ssm_k': _A_in['ssm_k'], 'A_ssm_D': _A_in['ssm_D'], 'B_x': _B_in['x'], 'B_w_in': _B_in['w_in'], 'B_w_sp': _B_in['w_sp'], 'B_b_sp': _B_in['b_sp'], 'B_w_out': _B_in['w_out']}

def reference(A_q, A_k, A_v, A_shift_k, A_ssm_k, A_ssm_D, B_x, B_w_in, B_w_sp, B_b_sp, B_w_out):

    def _A_ref(q, k, v, shift_k, ssm_k, ssm_D):
        B, S, D = q.shape
        ks = shift_k.shape[-1]
        k_pad = jnp.pad(k, ((0, 0), (ks - 1, 0), (0, 0)))
        k_shift = jnp.zeros_like(k)
        for t in range(ks):
            k_shift = k_shift + k_pad[:, t:t + S, :] * shift_k[:, ks - 1 - t][None, None, :]
        kv = k_shift * v
        L = 2 * S
        kv_pad = jnp.pad(kv, ((0, 0), (0, S), (0, 0)))
        kf_pad = jnp.pad(ssm_k, ((0, 0), (0, S)))
        kv_f = (lambda x, axes=(-2, -1): jnp.fft.rfft2(x.astype(jnp.float32), axes=axes))(kv_pad[:, None, :, :], axes=(1, 2))
        kf_f = (lambda x, axes=(-2, -1): jnp.fft.rfft2(x.astype(jnp.float32), axes=axes))(kf_pad[:, None, :], axes=(1, 2))
        kf_f = (lambda x, *d: x.transpose(*d))(kf_f, 1, 2, 0)
        y_f = kv_f * kf_f[None, :, :, :]
        y = (lambda x, s, axes=(-2, -1): jnp.fft.irfft2(x, s=s, axes=axes).astype(jnp.bfloat16))(y_f, (1, L), axes=(1, 2))[:, 0, :S, :]
        y = y + kv * ssm_D[None, None, :]
        return q * y

    def _B_ref(x, w_in, w_sp, b_sp, w_out):
        B, S, D = x.shape
        F = w_in.shape[-1]
        Fh = F // 2
        z = _gelu(jnp.einsum('bsd,df->bsf', x, w_in))
        z1 = z[..., :Fh].copy()
        z2 = _layernorm(z[..., Fh:], axis=-1)
        g = jnp.einsum('ts,bsf->btf', w_sp, z2) + b_sp[None, :, None]
        return jnp.einsum('bsf,fd->bsd', z1 * g, w_out)
    x = A_q
    x = x + _A_ref(_layernorm(x, axis=-1), A_k, A_v, A_shift_k, A_ssm_k, A_ssm_D)
    x = x + _B_ref(_layernorm(x, axis=-1), B_w_in, B_w_sp, B_b_sp, B_w_out)
    x = x + _A_ref(_layernorm(x, axis=-1), A_k, A_v, A_shift_k, A_ssm_k, A_ssm_D)
    x = x + _B_ref(_layernorm(x, axis=-1), B_w_in, B_w_sp, B_b_sp, B_w_out)
    return x
```

```python
import functools
import numpy as np
import jax
import jax.numpy as jnp
from jax import lax
import jax.experimental.pallas as pl
import jax.experimental.pallas.tpu as pltpu

S = 2048
D = 1024
F = 3584
FH = 1792
N1 = 128
R = 4
CB = N1 * R
NC = S // CB
NL = D // 128
TM = 256
NB = S // TM
RG = 16
EPS = 1e-5
BF = jnp.bfloat16
F32 = jnp.float32
U32 = jnp.uint32


def _pack_rows(a):
    b = np.asarray(jnp.asarray(a, BF)).view(np.uint16).astype(np.uint32)
    return b[..., 0::2, :] | (b[..., 1::2, :] << 16)


def _tables():
    k1 = np.concatenate([np.arange(0, N1, 2), np.arange(1, N1, 2)]).astype(np.float64)
    m = np.arange(N1, dtype=np.float64)
    fwd = np.zeros((R, 2 * N1, N1))
    for r in range(R):
        ang = np.pi * np.outer(2 * k1 + 1, R * m + r) / (2 * CB)
        re, im = np.cos(ang), -np.sin(ang)
        fwd[r] = np.stack([re.reshape(16, 8, N1), im.reshape(16, 8, N1)], axis=1).reshape(2 * N1, N1)
    inv = np.transpose(fwd, (0, 2, 1)) / CB
    inv = inv.reshape(R, N1, 2, N1).transpose(0, 2, 1, 3)
    perm = np.zeros((N1, N1))
    for r in range(R):
        for mm in range(N1 // R):
            perm[r * (N1 // R) + mm, R * mm + r] = 1.0
    return fwd, inv, perm


def _ln(x):
    m = jnp.mean(x, axis=-1, keepdims=True)
    xc = x - m
    v = jnp.mean(xc * xc, axis=-1, keepdims=True)
    return xc * lax.rsqrt(v + EPS)


def _gelu(x):
    c = np.float32(np.sqrt(2.0 / np.pi))
    inner = x * (c + (c * 0.044715) * (x * x))
    hx = 0.5 * x
    return hx + hx * jnp.tanh(inner)


def _dot(a, b):
    return jnp.dot(a, b, preferred_element_type=F32)


def _dot_nt(a, b):
    return lax.dot_general(a, b, (((1,), (1,)), ((), ())), preferred_element_type=F32)


def _bf(w):
    return pltpu.bitcast(w, BF)


PS = 2 * NC * R


def _kernel(q_hbm, k_hbm, v_hbm, sk_ref, h_hbm, dd_ref, win_hbm, wsp_hbm, bsp_ref, wout_hbm,
            fwd_ref, inv_ref, perm_ref, out_hbm,
            qb, kb, vb, hb, win, wsp, wout, kf, vf, SA, SB, y3, x, z1, z2a, z2b, zf, ob, tbl,
            sems, csems):
    kvh = []
    for j in range(NL):
        ls = pl.ds(j * 128, 128)
        c = [pltpu.make_async_copy(k_hbm.at[:, ls], kb.at[j], csems.at[3 * j]),
             pltpu.make_async_copy(v_hbm.at[:, ls], vb.at[j], csems.at[3 * j + 1]),
             pltpu.make_async_copy(h_hbm.at[ls, :], hb.at[ls, :], csems.at[3 * j + 2])]
        for cc in c:
            cc.start()
        kvh.append(c)
    cps = []
    for i, (src, dst) in enumerate([(win_hbm, win), (q_hbm, qb.at[0:S, :]), (wsp_hbm, wsp), (wout_hbm, wout)]):
        cp = pltpu.make_async_copy(src, dst, sems.at[i])
        cp.start()
        cps.append(cp)

    kf[0:8, :] = jnp.zeros((8, 128), F32)
    for i in range(16):
        tbl[i] = i * 16
    tbl[16] = S
    tbl[17] = TM
    for i in range(NB):
        tbl[18 + i] = i * TM

    def bfly_store(SP, base, V, dd=None):
        V = [v.reshape(16, 2, 8, 128) for v in V]
        re = [v[:, 0] for v in V]
        im = [v[:, 1] for v in V]
        if dd is not None:
            re[0] = re[0] + dd
        a = (re[0] + re[2], im[0] + im[2])
        b = (re[0] - re[2], im[0] - im[2])
        c = (re[1] + re[3], im[1] + im[3])
        d = (re[1] - re[3], im[1] - im[3])
        X = [(a[0] + c[0], a[1] + c[1]), (b[0] + d[1], b[1] - d[0]),
             (a[0] - c[0], a[1] - c[1]), (b[0] - d[1], b[1] + d[0])]
        for k2 in range(R):
            SP[base + k2] = jnp.stack(X[k2], axis=1).reshape(2 * N1, 128)

    def fwd_stage(j, q, SP):
        r0 = pl.multiple_of(q * CB, CB)
        sk = sk_ref[:, j * 128:(j + 1) * 128].astype(F32)
        perm = _bf(perm_ref[...])
        ht = [_dot_nt(perm, hb[j * 128:(j + 1) * 128, pl.ds(r0 + a * N1, N1)]).astype(BF) for a in range(R)]
        kf[pl.ds(r0 + 8, CB), :] = kb[j, pl.ds(r0, CB), :].astype(F32)
        vf[...] = vb[j, pl.ds(r0, CB), :].astype(F32)
        ko = {o: kf[pl.ds(r0 + 8 + o, N1, stride=R), :] for o in range(-3, R)}
        V = []
        for r in range(R):
            ks = ko[r] * sk[0:1, :]
            for i in range(1, 4):
                ks = ks + ko[r - i] * sk[i:i + 1, :]
            u = (ks * vf[pl.ds(r, N1, stride=R), :]).astype(BF)
            V.append(_dot(_bf(fwd_ref[r]), u))
        bfly_store(SP, q * R, V)
        w = N1 // R
        V = []
        for r in range(R):
            hr = jnp.concatenate([ht[a][r * w:(r + 1) * w] for a in range(R)], axis=0)
            V.append(_dot(_bf(fwd_ref[r]), hr))
        dd = dd_ref[:, j * 128:(j + 1) * 128].astype(F32) * (q == 0).astype(F32)
        bfly_store(SP, NC * R + q * R, V, dd=dd)

    def prod_pos(t, sgn, SP):
        t16 = pl.multiple_of(tbl[t], 16)
        rr = pl.ds(t16, 8)
        ri = pl.ds(t16 + 8, 8)
        t8 = pl.multiple_of(t * 8, 8)
        prev = None
        for c in range(NC):
            Q = []
            for k2 in range(R):
                acc = None
                for i in range(c + 1):
                    ur, ui = SP[i * R + k2, rr, :], SP[i * R + k2, ri, :]
                    hs = NC * R + (c - i) * R + k2
                    hr, hi = SP[hs, rr, :], SP[hs, ri, :]
                    pr = ur * hr - ui * hi
                    pi = ur * hi + ui * hr
                    acc = (pr, pi) if acc is None else (acc[0] + pr, acc[1] + pi)
                Q.append(acc)
            if prev is None:
                Pc = Q
            elif sgn > 0:
                Pc = [(Q[e][0] - prev[e][1], Q[e][1] + prev[e][0]) for e in range(R)]
            else:
                Pc = [(Q[e][0] + prev[e][1], Q[e][1] - prev[e][0]) for e in range(R)]
            prev = Q
            a = (Pc[0][0] + Pc[2][0], Pc[0][1] + Pc[2][1])
            b = (Pc[0][0] - Pc[2][0], Pc[0][1] - Pc[2][1])
            cc = (Pc[1][0] + Pc[3][0], Pc[1][1] + Pc[3][1])
            d = (Pc[1][0] - Pc[3][0], Pc[1][1] - Pc[3][1])
            W = [(a[0] + cc[0], a[1] + cc[1]), (b[0] - d[1], b[1] + d[0]),
                 (a[0] - cc[0], a[1] - cc[1]), (b[0] + d[1], b[1] - d[0])]
            for r in range(R):
                wv = pltpu.bitcast(jnp.concatenate(W[r], axis=0).astype(BF), F32)
                s = c * R + r
                SP[PS + s // 2, pl.ds((s % 2) * N1 + t8, 8), :] = wv

    def prod_stage(j, q, SP):
        for e in range(2):
            prod_pos(2 * q + e, 1, SP)
            prod_pos(2 * q + e + 8, -1, SP)

    def inv_stage(j, q, SP):
        r0 = pl.multiple_of(q * CB, CB)
        for r in range(R):
            p = SP[PS + q * 2 + r // 2, pl.ds((r % 2) * N1, N1), :]
            yr = (_dot(_bf(inv_ref[r, 0]), _bf(p[:N1 // 2])) + _dot(_bf(inv_ref[r, 1]), _bf(p[N1 // 2:])))
            y3[j, pl.ds(r0 + r, N1, stride=R), :] = yr

    bufs = [SA, SB]
    with jax.named_scope("conv"):
        for s in range(NL + 2):
            jf, jp, ji = s, s - 1, s - 2
            if jf < NL:
                for cc in kvh[jf]:
                    cc.wait()

            def body(q, carry, jf=jf, jp=jp, ji=ji):
                if 0 <= ji < NL:
                    inv_stage(ji, q, bufs[ji % 2])
                if jf < NL:
                    fwd_stage(jf, q, bufs[jf % 2])
                if 0 <= jp < NL:
                    prod_stage(jp, q, bufs[jp % 2])
                return carry
            lax.fori_loop(0, NC, body, 0)

    def row0(i):
        if isinstance(i, int):
            return i * TM
        return pl.multiple_of(i * TM, TM)

    def rows_of(i):
        return pl.ds(row0(i), TM)

    def ln_in(src, i, chain=True):
        outs = []
        for g in range(TM // RG):
            rows = pl.ds(row0(i) + g * RG, RG)
            xr = src[rows, :].astype(F32)
            yv = jnp.concatenate([y3[j, rows, :] for j in range(NL)], axis=1)
            x1 = xr + _ln(xr) * yv
            x[rows, :] = x1
            xo = _ln(x1)
            outs.append(xo.astype(BF))
            if chain and g < TM // RG - 1:
                src[pl.ds(pl.multiple_of(tbl[16], 16), RG), 0:128] = xo[:, 0:128].astype(src.dtype)
        return jnp.concatenate(outs, axis=0)

    def mm_in(xn, i, z2, chain=True):
        z2[rows_of(i), :] = _gelu(_dot(xn, win[:, FH:])).astype(BF)
        ro = pl.multiple_of(tbl[18 + i], TM) if chain else row0(i)
        for g in range(TM // RG):
            zo = _ln(z2[pl.ds(ro + g * RG, RG), :].astype(F32))
            z2[pl.ds(row0(i) + g * RG, RG), :] = zo.astype(BF)
        za = _gelu(_dot(xn, win[:, :FH]))
        z1[rows_of(i), :] = za.astype(BF)

    def phase_b(i, z2):
        rows = rows_of(i)
        g = _dot(wsp[rows, :], z2[...]) + bsp_ref[rows, :]
        t = (z1[rows, :].astype(F32) * g).astype(BF)
        return x[rows, :] + _dot(t, wout[...])

    cps[0].wait(); cps[1].wait()
    with jax.named_scope("l1a"):
        xn0 = ln_in(qb, 0, chain=False)

        def l1a(i, xn):
            xn_next = ln_in(qb, jnp.minimum(i + 1, NB - 1))
            mm_in(xn, i, z2a)
            return xn_next
        lax.fori_loop(0, NB, l1a, xn0)

    cps[2].wait(); cps[3].wait()
    with jax.named_scope("l1b2a"):
        x[rows_of(0), :] = phase_b(0, z2a)
        xn0 = ln_in(x, 0, chain=False)

        def l1b(i, xn):
            x[rows_of(i), :] = phase_b(i, z2a)
            xn_next = ln_in(x, i)
            mm_in(xn, i - 1, z2b)
            return xn_next
        xn7 = lax.fori_loop(1, NB, l1b, xn0)
        mm_in(xn7, NB - 1, z2b)

    def l2b(i, carry):
        rows = rows_of(i)
        x4 = phase_b(i, z2b)
        ob[rows, :] = x4.astype(BF)
        pltpu.make_async_copy(ob.at[rows, :], out_hbm.at[rows, :], sems.at[4]).start()
        return carry
    with jax.named_scope("l2b"):
        lax.fori_loop(0, NB, l2b, 0)
    pltpu.make_async_copy(ob, out_hbm, sems.at[4]).wait()


_FWD, _INV, _PERM = _tables()


@jax.jit
def pallas_interleave_layers__ssm_conv_h3__mixer_gmlp__prompt_kernel(
    A_q, A_k, A_v, A_shift_k, A_ssm_k, A_ssm_D, B_x, B_w_in, B_w_sp, B_b_sp, B_w_out,
):
    import ml_dtypes
    def pk(a):
        b = a.astype(ml_dtypes.bfloat16).view(np.uint16).astype(np.uint32)
        return jnp.asarray(b[..., 0::2, :] | (b[..., 1::2, :] << 16))
    fwd, inv, perm = pk(_FWD), pk(_INV), pk(_PERM)
    any_spec = pl.BlockSpec(memory_space=pl.ANY)
    vmem_spec = pl.BlockSpec(memory_space=pltpu.VMEM)
    out = pl.pallas_call(
        _kernel,
        out_shape=jax.ShapeDtypeStruct((S, D), BF),
        in_specs=[any_spec, any_spec, any_spec, vmem_spec, any_spec, vmem_spec, any_spec, any_spec,
                  vmem_spec, any_spec, vmem_spec, vmem_spec, vmem_spec],
        out_specs=any_spec,
        scratch_shapes=[
            pltpu.VMEM((S + 16, D), BF),
            pltpu.VMEM((NL, S, 128), BF),
            pltpu.VMEM((NL, S, 128), BF),
            pltpu.VMEM((D, S), BF),
            pltpu.VMEM((D, F), BF),
            pltpu.VMEM((S, S), BF),
            pltpu.VMEM((FH, D), BF),
            pltpu.VMEM((S + 8, 128), F32),
            pltpu.VMEM((CB, 128), F32),
            pltpu.VMEM((PS + NC * R // 2, 2 * N1, 128), F32),
            pltpu.VMEM((PS + NC * R // 2, 2 * N1, 128), F32),
            pltpu.VMEM((NL, S, 128), F32),
            pltpu.VMEM((S + 16, D), F32),
            pltpu.VMEM((S, FH), BF),
            pltpu.VMEM((S, FH), BF),
            pltpu.VMEM((S, FH), BF),
            pltpu.VMEM((TM + 8, FH), F32),
            pltpu.VMEM((S, D), BF),
            pltpu.SMEM((18 + NB,), jnp.int32),
            pltpu.SemaphoreType.DMA((5,)),
            pltpu.SemaphoreType.DMA((3 * NL,)),
        ],
        compiler_params=pltpu.CompilerParams(vmem_limit_bytes=120 * 1024 * 1024),
    )(A_q[0], A_k[0], A_v[0], A_shift_k.T, A_ssm_k, A_ssm_D.reshape(1, D), B_w_in, B_w_sp,
      B_b_sp.astype(F32).reshape(S, 1), B_w_out, fwd, inv, perm)
    return out[None]
```

```python
import functools
import numpy as np
import ml_dtypes
import jax
import jax.numpy as jnp
from jax import lax
import jax.experimental.pallas as pl
import jax.experimental.pallas.tpu as pltpu

S = 2048
D = 1024
FH = 1792
N1 = 128
R = 4
CB = N1 * R
NC = S // CB
NL = D // 128
TM = 256
NB = S // TM
RG = 16
EPS = 1e-5
BF = jnp.bfloat16
F32 = jnp.float32

PS = 2 * NC * R
SL = 2 * N1
W4 = N1 // R
O_FEN = 2 * PS * SL
O_TB = 0
T_I = R * N1
T_P = 2 * R * N1
T_END = T_P + N1 // 2
O_KF = 0
O_VF = 0
O_Y = 0
HB = S // 2
HP = HB + TM
NP = HB // TM
KH = D // 2
NH = FH // 2
YR = S
BIG_ROWS = O_FEN + 8
CH = 32
MORDER = "I0 I1 M U H"
T_PUSH = 40
T_WLEAD = 110
T_LEAD = 80
T_LAT = 130
T_SCALE = 100
UNR = 1
NFINE = 3
T_SLACK = 20
BG = 2
T_RES = 115
MGATE = 2
IDRAIN = 2
LA = 2
WSCHED = {2: (0,), 3: (1,), 4: (2,), 5: (3,), 6: (4, 5), 7: (6, 7)}
QS0 = 8
QS1 = 9
PLAG = True
STHR = True
SDRAIN = False
VLIM = 128
IGH = 4
WC = 256
LW = 256
IGA = 2
IGC = 2
LKS = (0,)*6+(1,)*4+(2,)*6+(3,)*4+(4,)*6+(7,)*4+(8,)*4+(9,)*2+(10,)*1
CKS = (0,)*6+(1,)*6+(2,)*6+(3,)*4+(4,)*2+(5,)*1
NKS = (7, 8, 9, 10, 11, 12)
AKS = (0, 2, 4, 9, 10, 11, 12)


def _tables():
    k1 = np.concatenate([np.arange(0, N1, 2), np.arange(1, N1, 2)]).astype(np.float64)
    m = np.arange(N1, dtype=np.float64)
    fwd = np.zeros((R, 2 * N1, N1))
    for r in range(R):
        ang = np.pi * np.outer(2 * k1 + 1, R * m + r) / (2 * CB)
        re, im = np.cos(ang), -np.sin(ang)
        fwd[r] = np.stack([re.reshape(16, 8, N1), im.reshape(16, 8, N1)], axis=1).reshape(2 * N1, N1)
    inv = np.transpose(fwd, (0, 2, 1)) / CB
    inv = inv.reshape(R, N1, 2, N1).transpose(0, 2, 1, 3)
    perm = np.zeros((N1, N1))
    for r in range(R):
        for mm in range(N1 // R):
            perm[r * (N1 // R) + mm, R * mm + r] = 1.0
    a = np.concatenate([fwd.reshape(-1, N1), inv.reshape(-1, N1), perm], axis=0)
    b = a.astype(ml_dtypes.bfloat16).view(np.uint16).astype(np.uint32)
    return (b[0::2, :] | (b[1::2, :] << 16)).view(np.float32)


def _gelu(x):
    c = np.float32(np.sqrt(2.0 / np.pi))
    inner = x * (c + (c * 0.044715) * (x * x))
    hx = 0.5 * x
    return hx + hx * jnp.tanh(inner)


def _dot(a, b):
    return jnp.dot(a, b, preferred_element_type=F32)


def _dot_nt(a, b):
    return lax.dot_general(a, b, (((1,), (1,)), ((), ())), preferred_element_type=F32)


def _mo(v, m):
    return v if isinstance(v, int) else pl.multiple_of(v, m)


def _bf(w):
    return pltpu.bitcast(w, BF)


def _kernel(q_hbm, k_hbm, v_hbm, sk_hbm, h_hbm, dd_hbm, win_hbm, wsp_hbm, bsp_hbm, wout_hbm,
            tb_hbm, out_hbm,
            qb, kvb, hb, win, wsp, wout, BIG, TB, KV, VF, Y3, UA, UB, PA, PB, x, zt, z2, xs, sk_ref, ddb, bsb, DD, BB, tbl,
            sems):
    OC, OW, OO, OF = 20, 20 + 3 * NL, 20 + 5 * NL, 20 + 5 * NL + 2 * NB
    def kvh_chunk(j, q):
        ls = pl.ds(j * 128, 128)
        rs = pl.ds(_mo(q * CB, CB), CB)
        n = (j * NC + q) * 3
        return [pltpu.make_async_copy(k_hbm.at[rs, ls], kvb.at[j, rs, :], sems.at[OF + n]),
                pltpu.make_async_copy(v_hbm.at[rs, ls], kvb.at[NL + j, rs, :], sems.at[OF + n + 1]),
                pltpu.make_async_copy(h_hbm.at[ls, rs], hb.at[ls, rs], sems.at[OF + n + 2])]
    kvh = []
    for j in range(NL):
        ls = pl.ds(j * 128, 128)
        if j < NFINE:
            kvh.append([c for q in range(NC) for c in kvh_chunk(j, q)])
        else:
            kvh.append([pltpu.make_async_copy(k_hbm.at[:, ls], kvb.at[j, 0:S, :], sems.at[OC + 3 * j]),
                        pltpu.make_async_copy(v_hbm.at[:, ls], kvb.at[NL + j, 0:S, :], sems.at[OC + 3 * j + 1]),
                        pltpu.make_async_copy(h_hbm.at[ls, :], hb.at[ls, :], sems.at[OC + 3 * j + 2])])
    wcp = [[pltpu.make_async_copy(win_hbm.at[pl.ds((n % 4 // 2) * KH, KH), pl.ds((1 - n // 4) * FH + (n % 2) * NH, NH)],
                                  win.at[7 * (n // 4) + 1 + n % 4], sems.at[OW + n])] for n in range(8)]
    qrs = [(HB - TM, HB), (HB - 2 * TM, HB - TM), (0, HB - 2 * TM)]
    qcp = [[pltpu.make_async_copy(q_hbm.at[h * HB + a:h * HB + b, :], qb.at[h, TM + a:TM + b, :], sems.at[10 + 2 * n + h])
            for h in range(2)] for n, (a, b) in enumerate(qrs)]
    cps = [pltpu.make_async_copy(wsp_hbm.at[pl.ds((n // 2) * HB + a, b - a), pl.ds((n % 2) * HB, HB)],
                                 wsp.at[(2, 4, 1, 3)[n], a:b, :], sems.at[so + n])
           for a, b, so in ((0, TM, 0), (TM, HB, OW + 8)) for n in range(4)] + [
        pltpu.make_async_copy(wout_hbm.at[pl.ds((n // 2) * NH, NH), pl.ds((n % 2) * KH, KH)], wout.at[1 + n, 0:NH, :], sems.at[16 + n])
        for n in range(4)]
    tcp = [pltpu.make_async_copy(tb_hbm.at[T_P:T_END, :], TB.at[T_P:T_END, :], sems.at[4]),
           pltpu.make_async_copy(tb_hbm.at[0:T_I, :], TB.at[0:T_I, :], sems.at[5]),
           pltpu.make_async_copy(tb_hbm.at[T_I:T_P, :], TB.at[T_I:T_P, :], sems.at[6])]
    scp = [pltpu.make_async_copy(bsp_hbm, bsb, sems.at[7]), pltpu.make_async_copy(sk_hbm, sk_ref, sems.at[8]),
           pltpu.make_async_copy(dd_hbm, ddb, sems.at[9])]
    tcp[0].start()
    for cc in scp:
        cc.start()
    for j in range(LA):
        for cc in kvh[j]:
            cc.start()
        if j == 0:
            tcp[1].start()

    KV[O_KF:O_KF + 8, :] = jnp.zeros((8, 128), F32)

    def zinit(j, carry):
        r = pl.multiple_of(j * 16, 16)
        Y3[pl.ds(r + O_Y, 16), :] = jnp.zeros((16, 128), F32)
        for h in range(2):
            qb[h, pl.ds(r, 16), :] = jnp.zeros((16, D), BF)
        return carry
    lax.fori_loop(0, 2 * NL, zinit, 0)
    for i in range(16):
        tbl[i] = i * 16
    tbl[17] = O_FEN
    tbl[26] = D
    tbl[27] = 0
    tbl[28] = T_END
    tbl[29] = S
    BIG[O_FEN:O_FEN + 8, :] = jnp.zeros((8, 128), F32)
    for wb in (UA, UB, PA, PB):
        wb[0, 0:16, :] = jnp.zeros((16, 128), BF)

    def gate_t(val):
        TB[pl.ds(pl.multiple_of(tbl[28], 8), 8), :] = val

    def gate_p(val):
        BIG[pl.ds(pl.multiple_of(tbl[17], 8), 8), :] = val

    def gate_s(val):
        kvb[0, pl.ds(pl.multiple_of(tbl[29], 16), 16), :] = jnp.concatenate([val, val], axis=0).astype(BF)

    def drain(wref):
        return wref[tbl[27], 0:16, :].astype(F32)[0:8]

    def gate_w(val, wref):
        v16 = jnp.concatenate([val, val], axis=0).astype(BF)
        if wref is hb:
            hb[pl.ds(pl.multiple_of(tbl[26], 16), 16), 0:128] = v16
        else:
            wref[tbl[27], 0:16, :] = v16

    def fwd_batch(j, q, UH, so, is_h):
        base = (NC * R if is_h else 0) + q * R

        def fin(lhs, w):
            V = [_dot(lhs[r], w[r]) for r in range(R)]
            dd = None
            if is_h and not (isinstance(q, int) and q > 0):
                dd = DD[j:j + 1, :]
                if not isinstance(q, int):
                    dd = dd * (q == 0).astype(F32)
            sv = BIG.at[pl.ds(_mo((so + base) * SL, SL), R * SL), :]

            def bf(g):
                for t in range(g * BG, (g + 1) * BG):
                    re = [v[16 * t:16 * t + 8] for v in V]
                    im = [v[16 * t + 8:16 * t + 16] for v in V]
                    if dd is not None:
                        re[0] = re[0] + dd
                    a = (re[0] + re[2], im[0] + im[2])
                    b = (re[0] - re[2], im[0] - im[2])
                    c = (re[1] + re[3], im[1] + im[3])
                    d = (re[1] - re[3], im[1] - im[3])
                    X = [(a[0] + c[0], a[1] + c[1]), (b[0] + d[1], b[1] - d[0]),
                         (a[0] - c[0], a[1] - c[1]), (b[0] - d[1], b[1] + d[0])]
                    for k2 in range(R):
                        sv[k2 * SL + 16 * t:k2 * SL + 16 * t + 8, :] = X[k2][0]
                        sv[k2 * SL + 16 * t + 8:k2 * SL + 16 * t + 16, :] = X[k2][1]
            return [(T_RES + 16 * BG * (g + 1) + T_SLACK, functools.partial(bf, g)) for g in range(16 // BG)]
        return (UH, lambda: [UH[1 + base + r] for r in range(R)], [r * N1 for r in range(R)], 4, fin)

    def perm_batch(j, q, UH):
        r0 = _mo(q * CB, CB)

        def fin(lhs, w):
            uv = UH.at[pl.ds(1 + q * R, NC * R + R)]
            ht = [_dot_nt(lhs[0], w[a]) for a in range(R)]

            def put(r):
                for a in range(R):
                    uv[NC * R + r, a * W4:(a + 1) * W4, :] = ht[a][r * W4:(r + 1) * W4].astype(BF)
                if MGATE and r % MGATE == MGATE - 1:
                    gate_t(drain(UH))
            return [(T_RES + W4 * (r + 1) + T_SLACK, functools.partial(put, r)) for r in range(R)]
        return (hb, lambda: [hb[j * 128:(j + 1) * 128, pl.ds(r0 + a * N1, N1)] for a in range(R)], [T_P], 2, fin)

    def inv_batch(j, q, PP, h, dr=True):
        rs = (2 * h, 2 * h + 1)

        def fin(lhs, w):
            yv = Y3.at[pl.ds(_mo(q * CB, CB) + (O_Y + j * YR + TM), CB), :]
            ys = [(_dot(lhs[2 * n], w[n][:N1]), _dot(lhs[2 * n + 1], w[n][N1:])) for n in range(2)]

            def put(g):
                for n, r in enumerate(rs):
                    yv[pl.ds(g * N1 + r, W4, stride=R), :] = (ys[n][0][g * W4:(g + 1) * W4]
                                                               + ys[n][1][g * W4:(g + 1) * W4])
                if dr and IDRAIN and g % IDRAIN == IDRAIN - 1:
                    gate_t(Y3[pl.ds(pl.multiple_of(tbl[27], 8), 8), :])
            return [(T_RES + W4 * (g + 1) + T_SLACK, functools.partial(put, g)) for g in range(R)]
        return (PP, lambda: [PP[1 + q * R + r] for r in rs],
                [T_I + r * N1 + hh * (N1 // 2) for r in rs for hh in range(2)], 2, fin)

    def sconv_gen(j, q, UH, clock):
        r0 = _mo(q * CB, CB)
        uv = UH.at[pl.ds(1 + q * R, NC * R + R)]
        kv_ = KV.at[pl.ds(r0 + O_KF, CB + 8), :]
        sk = sk_ref[:, j * 128:(j + 1) * 128].astype(F32)
        n = 16
        m = n * R
        na = N1 // n

        def stage(a):
            kv_[8 + a * m:8 + (a + 1) * m, :] = kvb[j, pl.ds(r0 + a * m, m), :].astype(F32)
            VF[O_VF + a * m:O_VF + (a + 1) * m, :] = kvb[NL + j, pl.ds(r0 + a * m, m), :].astype(F32)
        for a in range(na):
            if STHR and clock:
                gate_s(clock[-1])
            stage(a)
            yield (a + 0.25) / na, None
            ko = {o: kv_[pl.ds(8 + a * m + o, n, stride=R), :] for o in range(-3, R)}
            for r in range(R):
                ks = ko[r] * sk[0:1, :]
                for i in range(1, 4):
                    ks = ks + ko[r - i] * sk[i:i + 1, :]
                u = ks * VF[pl.ds(O_VF + a * m + r, n, stride=R), :]
                uv[r, a * n:(a + 1) * n, :] = u.astype(BF)
            yield (a + 1) / na, (drain(UH) if SDRAIN else u[8:])

    def prod_gen(q, so, PP, clock, n0):
        ops = 0
        tot = 4 * 392
        for e in range(4):
            sgn = 1 - 2 * (e % 2)
            t = 2 * q + e // 2 + 8 * (e % 2)
            sv = BIG.at[pl.ds(pl.multiple_of(tbl[t], 16) + so * SL, (PS - 1) * SL + 16), :]
            tp = _mo(t * 16, 16)
            prev = None
            for c in range(NC):
                Q = []
                for k2 in range(R):
                    acc = None
                    for i in range(c + 1):
                        us = (i * R + k2) * SL
                        hs = (NC * R + (c - i) * R + k2) * SL
                        ur, ui = sv[us:us + 8, :], sv[us + 8:us + 16, :]
                        hr, hi = sv[hs:hs + 8, :], sv[hs + 8:hs + 16, :]
                        pr = ur * hr - ui * hi
                        pi = ur * hi + ui * hr
                        acc = (pr, pi) if acc is None else (acc[0] + pr, acc[1] + pi)
                    Q.append(acc)
                    ops += 8 * c + 6
                    clock.append(acc[1])
                    yield ops / tot, acc[1]
                if PLAG and (e or c or n0):
                    gate_p(drain(PP))
                if prev is None:
                    Pc = Q
                elif sgn > 0:
                    Pc = [(Q[n][0] - prev[n][1], Q[n][1] + prev[n][0]) for n in range(R)]
                else:
                    Pc = [(Q[n][0] + prev[n][1], Q[n][1] - prev[n][0]) for n in range(R)]
                prev = Q
                a = (Pc[0][0] + Pc[2][0], Pc[0][1] + Pc[2][1])
                b = (Pc[0][0] - Pc[2][0], Pc[0][1] - Pc[2][1])
                cc = (Pc[1][0] + Pc[3][0], Pc[1][1] + Pc[3][1])
                d = (Pc[1][0] - Pc[3][0], Pc[1][1] - Pc[3][1])
                W = [(a[0] + cc[0], a[1] + cc[1]), (b[0] - d[1], b[1] + d[0]),
                     (a[0] - cc[0], a[1] - cc[1]), (b[0] + d[1], b[1] - d[0])]
                for r in range(R):
                    PP[1 + c * R + r, pl.ds(tp, 16), :] = jnp.concatenate(W[r], axis=0).astype(BF)
                if not PLAG:
                    gate_p(W[3][1])
                clock.append(W[3][1])
                ops += 20 if c == 0 else 28
                yield ops / tot, W[3][1]

    def wsum_gen(o, q):
        r0 = _mo(q * (KH // NC), KH // NC)
        steps = [(g, c) for g in range(KH // NC // 16) for c in range(0, NH, WC)]
        for n, (g, c) in enumerate(steps):
            r, cs = pl.ds(r0 + g * 16, 16), slice(c, min(c + WC, NH))
            b11, b12, b21, b22 = [win[o + 1 + k, r, cs].astype(F32) for k in range(4)]
            for k, v in ((0, b11 + b22), (2, b12 - b22), (3, b21 - b11), (5, b11 + b12), (6, b21 + b22)):
                win[o + k, r, cs] = v.astype(BF)
            yield (n + 1) / len(steps), None

    def emit(batches, gens):
        ev = []
        t0s = []
        t = T_PUSH
        for bi, bt in enumerate(batches):
            ev.append((t - T_WLEAD, bi, -1))
            t0s.append(t)
            for c in range(bt[3]):
                ev.append((t + 64 * c - T_LEAD, bi, c))
            t += 64 * bt[3]
        tend = t + T_LAT - T_SCALE
        ev.sort()
        st = [dict(l=[[] for _ in bt[2]]) for bt in batches]
        last = {}
        lastv = []

        def fire(now):
            while ev and ev[0][0] <= now:
                _, bi, c = ev.pop(0)
                bt = batches[bi]
                if c >= 100:
                    st[bi]["c"][c - 100]()
                elif c < 0:
                    if lastv:
                        gate_w(lastv[-1], bt[0])
                    st[bi]["w"] = bt[1]()
                else:
                    for v in last.values():
                        if v is not None and v is not False:
                            gate_t(v)
                    last.clear()
                    for n, off in enumerate(bt[2]):
                        o = O_TB + off + c * CH
                        st[bi]["l"][n].append(TB[o:o + CH, :])
                    if c == bt[3] - 1:
                        cons = bt[4]([_bf(jnp.concatenate(l, axis=0)) for l in st[bi]["l"]], st[bi]["w"])
                        st[bi]["c"] = [f for _, f in cons]
                        ev.extend((t0s[bi] + dt, bi, 100 + n) for n, (dt, _) in enumerate(cons))
                        ev.sort()
        fire(0)
        pos = [0.0] * len(gens)
        live = list(range(len(gens)))
        while live:
            g = min(live, key=lambda i: pos[i])
            try:
                pos[g], v = next(gens[g])
            except StopIteration:
                live.remove(g)
                continue
            if v is not None:
                last[g] = v
                lastv.append(v)
            fire(min(pos[i] for i in live) * tend)
        fire(1e9)

    tcp[0].wait()
    for cc in scp:
        cc.wait()
    DD[...] = ddb[...].astype(F32).reshape(NL, 128)
    bs = bsb[...].astype(F32).reshape(S // N1, N1)
    for c in range(S // N1):
        bc = _dot_nt(_bf(TB[T_P:T_END, :]), jnp.broadcast_to(bs[c:c + 1, :], (N1, N1)).astype(BF))
        for r in range(R):
            BB[pl.ds(c * N1 + r, W4, stride=R), :] = bc[r * W4:(r + 1) * W4]

    sbuf, ubuf, pbuf = [0, PS], [UA, UB], [PA, PB]
    with jax.named_scope("conv"):
        for s in range(NL + 2):
            jr, jf, jp, ji = s, s - 1, s - 2, s - 3
            if s in (1, 3):
                tcp[(s + 1) // 2].wait()
            if NFINE <= jr < NL:
                for cc in kvh[jr]:
                    cc.wait()
            if s + LA < NL:
                for cc in kvh[s + LA]:
                    cc.start()
            if s == 0:
                tcp[2].start()
            for n in WSCHED.get(s, ()):
                for cc in wcp[n]:
                    cc.start()
            if s == QS0:
                for cc in qcp[0] + qcp[1]:
                    cc.start()
            if s == QS1:
                for cc in cps[:4] + qcp[2]:
                    cc.start()

            if s >= NL:
                for cc in sum(wcp[4 * (s - NL):4 * (s - NL) + 4], []):
                    cc.wait()

            def body(qq, carry, jr=jr, jf=jf, jp=jp, ji=ji):
                hf, hi_, hr_, hp = 0 <= jf < NL, 0 <= ji < NL, jr < NL, 0 <= jp < NL
                qs = [qq * UNR + n for n in range(UNR)]
                if jr < NFINE:
                    for q in qs:
                        for cc in kvh_chunk(jr, q):
                            cc.wait()
                batches = []
                for q in qs:
                    for kind in MORDER.split():
                        if kind == "U" and hf:
                            batches.append(fwd_batch(jf, q, ubuf[jf % 2], sbuf[jf % 2], False))
                        if kind == "H" and hf:
                            batches.append(fwd_batch(jf, q, ubuf[jf % 2], sbuf[jf % 2], True))
                        if kind[0] == "I" and hi_:
                            batches.append(inv_batch(ji, q, pbuf[ji % 2], int(kind[1])))
                        if kind == "M" and hr_:
                            batches.append(perm_batch(jr, q, ubuf[jr % 2]))
                clock = []

                def chain(mk):
                    for n, q in enumerate(qs):
                        for p, v in mk(q, n):
                            yield (n + p) / UNR, v
                gens = []
                if hp:
                    gens.append(chain(lambda q, n: prod_gen(q, sbuf[jp % 2], pbuf[jp % 2], clock, n)))
                if hr_:
                    gens.append(chain(lambda q, n: sconv_gen(jr, q, ubuf[jr % 2], clock)))
                if jr >= NL:
                    gens.append(chain(lambda q, n: wsum_gen(7 * (jr - NL), q)))
                emit(batches, gens)
                return carry
            if UNR == NC:
                body(0, 0)
            else:
                lax.fori_loop(0, NC // UNR, body, 0)

    def row0(i):
        if isinstance(i, int):
            return i * TM
        return pl.multiple_of(i * TM, TM)

    def a_ops(a11, a12, a21, a22):
        return [a11 + a22, a21 + a22, a11, a22, a11 + a12, a21 - a11, a12 - a22]

    def b_ops(b11, b12, b21, b22):
        return [b11 + b22, b11, b12 - b22, b21 - b11, b22, b11 + b12, b21 + b22]

    def paced(steps, ks, nc=NH):
        nt = (TM // 8) * (nc // 128)
        zero = jnp.full((8, 128), tbl[27], jnp.int32)

        def after(k, m):
            for n, st in enumerate(steps):
                u = n * len(ks) * nt // len(steps)
                if ks[u // nt] == k:
                    t = (u - ks.index(k) * nt) // ks.count(k)
                    j, g = divmod(t, TM // 8)
                    tile = m[g * 8:(g + 1) * 8, j * 128:(j + 1) * 128]
                    zr = pltpu.bitcast(pltpu.bitcast(tile, jnp.int32) & zero, F32)
                    st(jnp.concatenate([zr, zr], axis=0))
        return after

    def ln_steps(sv, xw, base, xv, ig):
        st = {}

        def wide(v, zr):
            return jnp.concatenate([v + zr] * (LW // 128), axis=1)

        def fold(v):
            return sum([v[:, c:c + 128] for c in range(128, LW, 128)], v[:, 0:128])

        def step(ph, g, h, c, zr):
            gs = slice(g * RG, (g + 1) * RG)
            e = st.setdefault((g, h), {})
            v = (sv if ph < 3 else xw)[h, gs, c:c + LW].astype(F32)
            if ph == 0:
                p = fold(v) + zr
            elif ph == 2:
                yv = jnp.concatenate([Y3[pl.ds(base + (O_Y + j * YR + h * HB + g * RG), RG), :]
                                      for j in range(c // 128, (c + LW) // 128)], axis=1)
                v = v + (v - wide(e["m"], zr)) * e["r"] * yv
                xw[h, gs, c:c + LW] = v
                p = fold(v)
            else:
                v = v - wide(e["m"], zr)
                p = fold(v * v)
            e["a"] = p if c == 0 else e["a"] + p
            if c + LW == D:
                t = jnp.sum(e["a"], axis=-1, keepdims=True) * (1.0 / D)
                if ph % 2:
                    e["r"] = lax.rsqrt(t + EPS)
                else:
                    e["m"] = t

        def last(g, c, zr):
            gs = slice(g * RG, (g + 1) * RG)
            mz = [st[g, h]["m"] + zr for h in range(2)]
            ops = a_ops(*[(xw[n // 2, gs, (n % 2) * KH + c:(n % 2) * KH + c + 128] - mz[n // 2]) * st[g, n // 2]["r"]
                          for n in range(4)])
            for n in range(7):
                xv[n, gs, c:c + 128] = ops[n].astype(BF)
        out = []
        for g0 in range(0, TM // RG, ig):
            out += [functools.partial(step, ph, g, h, c) for ph in range(4) for g in range(g0, g0 + ig)
                    for h in range(2) for c in range(0, D, LW)]
            out += [functools.partial(last, g, c) for g in range(g0, g0 + ig) for c in range(0, KH, 128)]
        return out

    def rview(ref, base):
        return ref.at[:, pl.ds(base, 2 * TM), :]

    def xview(base):
        return xs.at[:, pl.ds(base, 2 * TM), :]

    def mm_in(i, xv, hooks=(), order=(2, 4, 1, 3, 0, 5, 6, 9, 11, 8, 10, 7, 12, 13), nks=NKS):
        base = row0(i)
        rows = pl.ds(base, TM)
        hooks = list(hooks)
        ps, sts, m, done = {}, {}, {}, set()
        comb = {1: ((2, 1), (4, 1)), 2: ((1, 1), (3, 1)), 3: ((0, 1), (1, -1), (2, 1), (5, 1)),
                0: ((0, 1), (3, 1), (4, -1), (6, 1))}

        def norm(g, c0, zr):
            c1 = c0 + 128
            gs = slice(g * RG, (g + 1) * RG)
            r = pl.ds(base + g * RG, RG)
            if g not in sts:
                sts[g] = []
                for u in (0, 2):
                    mu = jnp.sum(ps[u][0][gs] + ps[u + 1][0][gs], axis=-1, keepdims=True) * (1.0 / FH)
                    e2 = jnp.sum(ps[u][1][gs] + ps[u + 1][1][gs], axis=-1, keepdims=True) * (1.0 / FH)
                    sts[g].append((mu, lax.rsqrt(jnp.maximum(e2 - mu * mu, 0.0) + EPS)))
            st = [(mu + zr, rs) for mu, rs in sts[g]]
            ops = b_ops(*[(z2[1 + n, r, c0:c1].astype(F32) - st[n // 2][0]) * st[n // 2][1] for n in range(4)])
            for n in range(7):
                z2[n, r, c0:c1] = ops[n].astype(BF)
        hooks.append(paced([functools.partial(norm, g, c) for g in range(TM // RG) for c in range(0, NH, 128)], nks))
        for k, p in enumerate(order):
            m[p] = tk = _dot(xv[p % 7, TM:2 * TM, :], win[p])
            o = p - p % 7
            fin = []
            for qd, terms in comb.items():
                if (o, qd) not in done and all(o + n in m for n, _ in terms):
                    done.add((o, qd))
                    v = m[o + terms[0][0]]
                    for n, sg in terms[1:]:
                        v = v + m[o + n] if sg > 0 else v - m[o + n]
                    fin.append((qd, v))
                    if len(terms) == 4:
                        tk = v
            for hk in hooks:
                hk(k, tk)
            for qd, v in fin:
                if o == 0:
                    v = _gelu(v)
                    bl = [v[:, c:c + 128] for c in range(0, NH, 128)]
                    ps[qd] = (sum(bl[1:], bl[0]), sum([b * b for b in bl[1:]], bl[0] * bl[0]))
                    z2[1 + qd, rows, :] = v.astype(BF)
                else:
                    zt[(2, 4, 1, 3)[qd], rows, :] = v.astype(BF)

    def wsp_ops(w, r, c, zr):
        a = [w[n, r, c:c + 128].astype(F32) for n in (2, 4, 1, 3)]
        ops = a_ops(a[0] + zr, a[1], a[2], a[3] + zr)
        for n in (0, 1, 4, 5, 6):
            w[n, r, c:c + 128] = ops[n].astype(BF)

    def wt_ops(w, o, r, c, zr):
        b = [w[o + 1 + n, r, c:c + 128].astype(F32) for n in range(4)]
        ops = b_ops(b[0] + zr, b[1], b[2], b[3] + zr)
        for n in (0, 2, 3, 5, 6):
            w[o + n, r, c:c + 128] = ops[n].astype(BF)

    def phase_b1(i, first):
        base = row0(i)
        rows = pl.ds(base, TM)
        rows2 = pl.ds(base + HB, TM)
        zv = zt.at[:, rows, :]
        cnt = [0]
        if first:
            w0 = pl.multiple_of(i * (NH // NP), 32)
            hk = paced([functools.partial(wt_ops, wout, 0, pl.ds(w0 + g * 16, 16), c)
                        for g in range(NH // NP // 16) for c in range(0, KH, 128)], (0, 1))

        def za(n):
            return _gelu(zv[n].astype(F32))

        def mm(n):
            m = _dot(wsp[n, rows, :], z2[n])
            if first:
                hk(cnt[0], m)
            cnt[0] += 1
            return m
        b1 = jnp.concatenate([BB[rows, :]] * (NH // 128), axis=1)
        b2 = jnp.concatenate([BB[rows2, :]] * (NH // 128), axis=1)
        m2 = mm(2)
        m3 = mm(3)
        m4 = mm(4)
        t12 = za(4) * (m2 + m4 + b1)
        m1 = mm(1)
        t21 = za(1) * (m1 + m3 + b2)
        m0 = mm(0)
        t22 = za(3) * (m0 - m1 + m2 + b2 + mm(5))
        t11 = za(2) * (m0 + m3 - m4 + b1 + mm(6))
        ops = a_ops(t11, t12, t21, t22)
        for n in range(7):
            zv[n] = ops[n].astype(BF)

    def phase_b2(i, xw, put, hk=None):
        rows = pl.ds(row0(i), TM)
        xr = slice(TM, 2 * TM)

        def mm(n):
            return _dot(zt[n, rows, :], wout[n])

        def tick(k, m):
            if hk is not None:
                hk(k, m)
            return m
        m2 = tick(0, mm(2))
        m4 = tick(1, mm(4))
        put(1, xw[0, xr, KH:] + m2 + m4)
        m1 = tick(2, mm(1))
        m3 = tick(3, mm(3))
        put(2, xw[1, xr, :KH] + m1 + m3)
        m0 = tick(4, mm(0))
        put(3, tick(5, xw[1, xr, KH:] + m0 - m1 + m2 + mm(5)))
        put(0, xw[0, xr, :KH] + m0 + m3 - m4 + mm(6))

    for cc in qcp[0]:
        cc.wait()
    with jax.named_scope("l1h"):
        for q in range(NC - 1, -1, -1):
            emit([inv_batch(NL - 1, q, pbuf[(NL - 1) % 2], h, False) for h in range(2)], [])
        hs = slice(NP * TM, (NP + 1) * TM)
        for st in ln_steps(qb.at[:, hs, :], x.at[:, hs, :], NP * TM, xs.at[:, hs, :], IGH):
            st(jnp.zeros((16, 128), F32))
    with jax.named_scope("l1a"):
        for cc in qcp[1] + cps[:4]:
            cc.wait()
        for cc in cps[4:]:
            cc.start()

    def l1a(n, carry):
        @pl.when(n == 1)
        def _():
            for cc in qcp[2] + cps[4:8]:
                cc.wait()
        i = NP - 1 - n
        xv = xview(row0(i))
        mm_in(i, xv, [paced(ln_steps(rview(qb, row0(i)), rview(x, row0(i)), row0(i), xv, IGA), LKS),
                      paced([functools.partial(wsp_ops, wsp, pl.ds(row0(n) + g * RG, RG), c)
                             for g in range(TM // RG) for c in range(0, HB, 128)], AKS)])
        return carry
    with jax.named_scope("l1l"):
        lax.fori_loop(0, NP, l1a, 0)

    for cc in cps[8:]:
        cc.wait()
    with jax.named_scope("l1b"):
        def l1b1(i, carry):
            phase_b1(i, True)
            return carry
        lax.fori_loop(0, NP, l1b1, 0)

    def l1b2(i, hk):
        xw = rview(x, row0(i))

        def put(n, v):
            xw[n // 2, TM:2 * TM, (n % 2) * KH:(n % 2 + 1) * KH] = v
        phase_b2(i, xw, put, hk)
        return 0
    with jax.named_scope("l1c"):
        lax.fori_loop(1, NP, lambda i, carry: l1b2(i, None), 0)
        xl = x.at[:, hs, :]
        l1b2(0, paced(ln_steps(xl, xl, NP * TM, xs.at[:, hs, :], IGC), CKS, KH))

    def l2a(n, carry):
        i = NP - 1 - n
        xv = xview(row0(i))
        xw = rview(x, row0(i))
        mm_in(i, xv, [paced(ln_steps(xw, xw, row0(i), xv, IGA), LKS)])
        return carry
    with jax.named_scope("l2a"):
        lax.fori_loop(0, NP, l2a, 0)

    with jax.named_scope("l2b"):
        def l2b1(i, carry):
            phase_b1(i, False)
            return carry
        lax.fori_loop(0, NP, l2b1, 0)

    def ocp(i, n):
        cols = pl.ds((n % 2) * KH, KH)
        return pltpu.make_async_copy(qb.at[n // 2, pl.ds(row0(i), TM), cols],
                                     out_hbm.at[pl.ds(row0(i) + (n // 2) * HB, TM), cols], sems.at[OO + 4 * i + n])

    def l2b2(i, carry):
        def put(n, v):
            qb[n // 2, pl.ds(row0(i), TM), (n % 2) * KH:(n % 2 + 1) * KH] = v.astype(BF)
            ocp(i, n).start()
        phase_b2(i, rview(x, row0(i)), put)
        return carry
    with jax.named_scope("l2c"):
        lax.fori_loop(0, NP, l2b2, 0)
    for i in range(NP):
        for n in range(4):
            ocp(i, n).wait()


_TB = _tables()


@jax.jit
def pallas_interleave_layers__ssm_conv_h3__mixer_gmlp__prompt_kernel(
    A_q, A_k, A_v, A_shift_k, A_ssm_k, A_ssm_D, B_x, B_w_in, B_w_sp, B_b_sp, B_w_out,
):
    any_spec = pl.BlockSpec(memory_space=pl.ANY)
    out = pl.pallas_call(
        _kernel,
        out_shape=jax.ShapeDtypeStruct((S, D), BF),
        in_specs=[any_spec] * 11,
        out_specs=any_spec,
        scratch_shapes=[
            pltpu.VMEM((2, HP, D), BF),
            pltpu.VMEM((2 * NL, S + 16, 128), BF),
            pltpu.VMEM((D + 16, S), BF),
            pltpu.VMEM((14, KH, NH), BF),
            pltpu.VMEM((7, HB, HB), BF),
            pltpu.VMEM((7, NH, KH), BF),
            pltpu.VMEM((BIG_ROWS, 128), F32),
            pltpu.VMEM((T_END + 8, 128), F32),
            pltpu.VMEM((S + 8, 128), F32),
            pltpu.VMEM((CB, 128), F32),
            pltpu.VMEM((NL * YR + TM, 128), F32),
            pltpu.VMEM((PS + 1, N1, 128), BF),
            pltpu.VMEM((PS + 1, N1, 128), BF),
            pltpu.VMEM((NC * R + 1, 2 * N1, 128), BF),
            pltpu.VMEM((NC * R + 1, 2 * N1, 128), BF),
            pltpu.VMEM((2, HP, D), F32),
            pltpu.VMEM((7, HB, NH), BF),
            pltpu.VMEM((7, HB, NH), BF),
            pltpu.VMEM((7, HP, KH), BF),
            pltpu.VMEM((4, D), BF),
            pltpu.VMEM((D,), BF),
            pltpu.VMEM((S,), BF),
            pltpu.VMEM((NL, 128), F32),
            pltpu.VMEM((S, 128), F32),
            pltpu.SMEM((30,), jnp.int32),
            pltpu.SemaphoreType.DMA((20 + 5 * NL + 2 * NB + 3 * NC * NFINE,)),
        ],
        compiler_params=pltpu.CompilerParams(vmem_limit_bytes=VLIM * 1024 * 1024),
    )(A_q[0], A_k[0], A_v[0], A_shift_k.T, A_ssm_k, A_ssm_D, B_w_in, B_w_sp,
      B_b_sp, B_w_out, jnp.asarray(_TB))
    return out[None]
```
